```python
import jax
import jax.numpy as jnp

def _softmax(x, axis=-1):
    return jax.nn.softmax(x, axis=axis)
def _gelu(x):
    return jax.nn.gelu(x, approximate=True)
def _silu(x):
    return jax.nn.silu(x)
def _sigmoid(x):
    return jax.nn.sigmoid(x)
def _layernorm(x, axis=-1, eps=1e-5):
    m = jnp.mean(x, axis=axis, keepdims=True)
    v = jnp.var(x, axis=axis, keepdims=True)
    return (x - m) / jnp.sqrt(v + eps)
def _scatter_add(tgt, idx, src, axis=0):
    return tgt.at[idx].add(src)
def _segment_sum(src, seg, n):
    return jax.ops.segment_sum(src, seg, n)
class _Rng:
    def __init__(self, key):
        self._k = key
    def _next(self):
        self._k, sub = jax.random.split(self._k)
        return sub
    def normal(self, shape):
        return jax.random.normal(self._next(), shape, dtype=jnp.bfloat16)
    def randint(self, lo, hi, shape):
        return jax.random.randint(self._next(), shape, lo, hi, dtype=jnp.int32)
    def uniform(self, shape, lo=0.0, hi=1.0):
        return jax.random.uniform(self._next(), shape, jnp.bfloat16, lo, hi)
    def permutation(self, n):
        return jax.random.permutation(self._next(), n)


kernel_name = 'concat_heads__gqa_block_cached__gqa_block_cached__near_ridge'

def setup_inputs():
    _rng = _Rng(jax.random.key(int.from_bytes(__import__("os").urandom(4), "little")))
    _w = (lambda a: (lambda t: t.astype(jnp.bfloat16) if jnp.issubdtype(t.dtype, jnp.floating) else t)(jnp.asarray(a)))
    def _A_setup():
        B, Sq, D = 8, 256, 640
        Hq, Hkv, Sk, Dh = 32, 32, 1024, 192
        assert Hq % Hkv == 0, (Hq, Hkv)
        return {
            "x": _w((lambda *s: _rng.normal(s) * 0.05)(B, Sq, D)),
            "k_cache": _w((lambda *s: _rng.normal(s) * 0.05)(B, Hkv, Sk, Dh)),
            "v_cache": _w((lambda *s: _rng.normal(s) * 0.05)(B, Hkv, Sk, Dh)),
            "wq": _w((lambda *s: _rng.normal(s) * 0.05)(D, Hq * Dh) * (D ** -0.5)),
            "wo": _w((lambda *s: _rng.normal(s) * 0.05)(Hq * Dh, D) * ((Hq * Dh) ** -0.5)),
        }
    _A_in = _A_setup()

    def _B_setup():
        B, Sq, D = 8, 256, 640
        Hq, Hkv, Sk, Dh = 32, 32, 1024, 192
        assert Hq % Hkv == 0, (Hq, Hkv)
        return {
            "x": _w((lambda *s: _rng.normal(s) * 0.05)(B, Sq, D)),
            "k_cache": _w((lambda *s: _rng.normal(s) * 0.05)(B, Hkv, Sk, Dh)),
            "v_cache": _w((lambda *s: _rng.normal(s) * 0.05)(B, Hkv, Sk, Dh)),
            "wq": _w((lambda *s: _rng.normal(s) * 0.05)(D, Hq * Dh) * (D ** -0.5)),
            "wo": _w((lambda *s: _rng.normal(s) * 0.05)(Hq * Dh, D) * ((Hq * Dh) ** -0.5)),
        }
    _B_in = _B_setup()

    return {
        "A_x": _A_in["x"],
        "A_k_cache": _A_in["k_cache"],
        "A_v_cache": _A_in["v_cache"],
        "A_wq": _A_in["wq"],
        "A_wo": _A_in["wo"],
        "B_x": _B_in["x"],
        "B_k_cache": _B_in["k_cache"],
        "B_v_cache": _B_in["v_cache"],
        "B_wq": _B_in["wq"],
        "B_wo": _B_in["wo"],
    }

def reference(A_x, A_k_cache, A_v_cache, A_wq, A_wo, B_x, B_k_cache, B_v_cache, B_wq, B_wo):
    def _A_ref(x, k_cache, v_cache, wq, wo):
        B, Sq, D = x.shape
        Hq, Dh = 32, 192
        Hkv = k_cache.shape[1]
        rep = Hq // Hkv
        q = (lambda x, *d: x.transpose(*d))((x @ wq).reshape(B, Sq, Hq, Dh), 0, 2, 1, 3)
        k = jnp.repeat(k_cache, rep, axis=1)
        v = jnp.repeat(v_cache, rep, axis=1)
        scores = jnp.einsum("bhqd,bhkd->bhqk", q, k) * (Dh ** -0.5)
        p = _softmax(scores, axis=-1)
        o = jnp.einsum("bhqk,bhkd->bhqd", p, v)
        return (lambda x, *d: x.transpose(*d))(o, 0, 2, 1, 3).reshape(B, Sq, Hq * Dh) @ wo

    def _B_ref(x, k_cache, v_cache, wq, wo):
        B, Sq, D = x.shape
        Hq, Dh = 32, 192
        Hkv = k_cache.shape[1]
        rep = Hq // Hkv
        q = (lambda x, *d: x.transpose(*d))((x @ wq).reshape(B, Sq, Hq, Dh), 0, 2, 1, 3)
        k = jnp.repeat(k_cache, rep, axis=1)
        v = jnp.repeat(v_cache, rep, axis=1)
        scores = jnp.einsum("bhqd,bhkd->bhqk", q, k) * (Dh ** -0.5)
        p = _softmax(scores, axis=-1)
        o = jnp.einsum("bhqk,bhkd->bhqd", p, v)
        return (lambda x, *d: x.transpose(*d))(o, 0, 2, 1, 3).reshape(B, Sq, Hq * Dh) @ wo

    a = _A_ref(A_x, A_k_cache, A_v_cache, A_wq, A_wo)
    b = _B_ref(B_x, B_k_cache, B_v_cache, B_wq, B_wo)
    return jnp.concatenate([a, b], axis=-1)
```

```python
import functools, math
import numpy as np
import jax, jax.numpy as jnp
from jax import lax
import jax.experimental.pallas as pl
import jax.experimental.pallas.tpu as pltpu

B,SQ,D,H,SK,DH = 8,256,640,32,1024,192
NT = (((1,),(1,)),((),()))
f32=jnp.float32; bf=jnp.bfloat16

def make(order, pv_mode='T', npairs=1, lsum='mxu', vmem=100, flags=None):
    G = 2*npairs
    NS = H//G
    c = (DH**-0.5)*math.log2(math.e)
    toks = order.split()
    def kernel(xa,xb,ka,va,kb,vb,wqa,wqb,woa,wob,o_ref,acc_ref):
        hp = pl.program_id(0); b = pl.program_id(1)
        @pl.when(hp==0)
        def _():
            acc_ref[b] = jnp.zeros((SQ,2*D),f32)
        R = ((xa,ka,va,wqa,woa),(xb,kb,vb,wqb,wob))
        q={}; S={}; O={}; P={}
        for t in toks:
            op=t[0]; i=int(t[1:])
            if op=='Q':
                s=i%2; pr=i//2
                x=R[s][0][b]
                qq = jnp.dot(x, R[s][3][:, pr*384:(pr+1)*384], preferred_element_type=f32)
                q[i]=(qq*c).astype(bf)
            elif op=='K':
                p=i//2; j=i%2; s=p%2; pr=p//2
                kT = R[s][1][0,2*pr+j]
                z = jnp.zeros((64,SK),bf)
                if j==0:
                    rhs = jnp.concatenate([kT,z],0); lhs=q[p][:,0:256]
                else:
                    rhs = jnp.concatenate([z,kT],0); lhs=q[p][:,128:384]
                S[i] = jnp.dot(lhs,rhs,preferred_element_type=f32)
            elif op=='S':
                sc=S.pop(i)
                m = jnp.max(sc,axis=1,keepdims=True)
                pf = jnp.exp2(sc-m)
                if pv_mode=='T' and lsum=='mxu':
                    P[i]=(pf.astype(bf),None)
                else:
                    P[i]=(pf.astype(bf), jnp.sum(pf,axis=1,keepdims=True))
            elif op=='P':
                p_=i//2; j=i%2; s=p_%2; pr=p_//2
                p,l = P.pop(i)
                vT = R[s][2][0,2*pr+j]
                if pv_mode=='T':
                    if lsum=='mxu':
                        vTe = jnp.concatenate([vT, jnp.ones((16,SK),bf)],0)
                        oT = lax.dot_general(vTe,p,NT,preferred_element_type=f32)
                        O[i]=(oT[:DH]*(1.0/oT[DH:DH+1])).astype(bf)
                    else:
                        oT = lax.dot_general(vT,p,NT,preferred_element_type=f32)
                        lT = jnp.broadcast_to(1.0/l,(SQ,128)).T[0:1,:]
                        O[i]=(oT*lT).astype(bf)
                else:
                    o = lax.dot_general(p,vT,NT,preferred_element_type=f32)
                    O[i]=(o*(1.0/l)).astype(bf)
            elif op=='O':
                s=i%2; pr=i//2
                if pv_mode=='T':
                    o = jnp.concatenate([O.pop(2*i),O.pop(2*i+1)],0).T
                else:
                    o = jnp.concatenate([O.pop(2*i),O.pop(2*i+1)],1)
                r = jnp.dot(o, R[s][4][pr*384:(pr+1)*384,:], preferred_element_type=f32)
                acc_ref[b,:,s*D:(s+1)*D] += r
        @pl.when(hp==NS-1)
        def _():
            o_ref[0] = acc_ref[b].astype(bf)

    kv_spec = pl.BlockSpec((1,G,DH,SK), lambda hp,b:(b,hp,0,0))
    x_spec = pl.BlockSpec((B,SQ,D), lambda hp,b:(0,0,0))
    wq_spec = pl.BlockSpec((D,G*DH), lambda hp,b:(0,hp))
    wo_spec = pl.BlockSpec((G*DH,D), lambda hp,b:(hp,0))
    def fn(ax,ak,av,awq,awo,bx,bk,bv,bwq,bwo):
        T = lambda a: jnp.swapaxes(a,2,3)
        return pl.pallas_call(kernel,
            grid=(NS,B),
            in_specs=[x_spec,x_spec,kv_spec,kv_spec,kv_spec,kv_spec,wq_spec,wq_spec,wo_spec,wo_spec],
            out_specs=pl.BlockSpec((1,SQ,2*D), lambda hp,b:(jnp.where(hp==NS-1,b,0),0,0)),
            out_shape=jax.ShapeDtypeStruct((B,SQ,2*D),bf),
            scratch_shapes=[pltpu.VMEM((B,SQ,2*D),f32)],
            compiler_params=pltpu.CompilerParams(dimension_semantics=('arbitrary','arbitrary'), vmem_limit_bytes=vmem*1024*1024, flags=flags),
        )(ax,bx,T(ak),T(av),T(bk),T(bv),awq,bwq,awo,bwo)
    return fn

seq1 = "Q0 K0 S0 P0 K1 S1 P1 O0 Q1 K2 S2 P2 K3 S3 P3 O1"
sw1  = "Q0 K0 K1 S0 P0 Q1 S1 K2 P1 S2 K3 O0 P2 S3 P3 O1"
sw2  = "Q0 K0 Q1 S0 K2 P0 S2 K1 P2 S1 K3 P1 S3 O0 P3 O1"
def swn(n):
    t=["Q0","K0"]
    U=4*n
    for u in range(U):
        nxt=u+1
        if nxt<U:
            if nxt%2==0: t.append(f"Q{nxt//2}")
            t.append(f"K{nxt}")
        t.append(f"S{u}")
        if u%2==0 and u>0: t.append(f"O{u//2-1}")
        t.append(f"P{u}")
    t.append(f"O{U//2-1}")
    return " ".join(t)

_fn = make(swn(2),'T',2,'mxu')

@jax.jit
def pallas_concat_heads__gqa_block_cached__gqa_block_cached__near_ridge_kernel(
    A_x, A_k_cache, A_v_cache, A_wq, A_wo, B_x, B_k_cache, B_v_cache, B_wq, B_wo):
    return _fn(A_x, A_k_cache, A_v_cache, A_wq, A_wo, B_x, B_k_cache, B_v_cache, B_wq, B_wo)
```

```python
import math
import jax
import jax.numpy as jnp
from jax import lax
import jax.experimental.pallas as pl
import jax.experimental.pallas.tpu as pltpu

B, SQ, D, H, SK, DH = 8, 256, 640, 32, 1024, 192
W = 2 * DH
NS = H // 2
T = NS * B
NT = (((1,), (1,)), ((), ()))
f32 = jnp.float32
bf = jnp.bfloat16
C = (DH ** -0.5) * math.log2(math.e)
ORDER = "Q0 K0 K1 Q1 K2 S0 P0 K3 S1 P1 S2 P2 S3 P3 O0 O1".split()


def _kernel(xa, xb, ka, va, kb, vb, wqa, wqb, woa, wob, o_hbm,
            xbuf, kbuf, vbuf, wqbuf, wobuf, acc_ref, obuf, xsem, kvsem, wsem, osem):
    X = (xa, xb); K = (ka, kb); V = (va, vb); WQ = (wqa, wqb); WO = (woa, wob)

    def kv_copy(t, s, kv):
        hp = t // B; b = t % B; sl = t % 2
        return pltpu.make_async_copy((K, V)[kv][s].at[b, pl.ds(hp * 2, 2)],
                                     (kbuf, vbuf)[kv].at[sl, s], kvsem.at[sl, s, kv])

    def woff(hp):
        return hp * W if isinstance(hp, int) else pl.multiple_of(hp * W, 128)

    def wq_copy(hp, s):
        return pltpu.make_async_copy(WQ[s].at[:, pl.ds(woff(hp), W)], wqbuf.at[hp % 2, s], wsem.at[hp % 2, s, 0])

    def wo_copy(hp, s):
        return pltpu.make_async_copy(WO[s].at[pl.ds(woff(hp), W), :], wobuf.at[hp % 2, s], wsem.at[hp % 2, s, 1])

    def x_copy(s, first):
        sl = pl.ds(0, 1) if first else pl.ds(1, B - 1)
        return pltpu.make_async_copy(X[s].at[sl], xbuf.at[s, sl], xsem.at[s, 0 if first else 1])

    def o_copy(b):
        return pltpu.make_async_copy(obuf.at[b], o_hbm.at[b], osem.at[b])

    def kv_start(t):
        for s in range(2):
            for kv in range(2):
                kv_copy(t, s, kv).start()

    def body(hp, b, first):
        t = hp * B + b; sl = t % 2; ws = hp % 2
        if not first:
            for s in range(2):
                for kv in range(2):
                    kv_copy(t, s, kv).wait()
            pl.when(t + 1 < T)(lambda: kv_start(t + 1))
        q = {}; S = {}; P = {}; O = {}
        for tk in ORDER:
            op = tk[0]; i = int(tk[1:])
            if first:
                if tk == "K0":
                    kv_copy(0, 0, 0).wait(); kv_copy(0, 1, 1).start()
                    for s in range(2): wo_copy(0, s).start()
                    kv_start(1)
                    for s in range(2): x_copy(s, False).start()
                elif tk == "Q1":
                    x_copy(1, True).wait(); wq_copy(0, 1).wait()
                elif tk == "K2": kv_copy(0, 1, 0).wait()
                elif tk == "P0": kv_copy(0, 0, 1).wait()
                elif tk == "P2": kv_copy(0, 1, 1).wait()
                elif tk == "O0":
                    for s in range(2): wo_copy(0, s).wait()
            if op == "Q":
                qq = jnp.dot(xbuf[i, b], wqbuf[ws, i], preferred_element_type=f32)
                q[i] = (qq * C).astype(bf)
            elif op == "K":
                s = i // 2; j = i % 2
                kT = kbuf[sl, s, j]
                z = jnp.zeros((64, SK), bf)
                if j == 0:
                    rhs = jnp.concatenate([kT, z], 0); lhs = q[s][:, 0:256]
                else:
                    rhs = jnp.concatenate([z, kT], 0); lhs = q[s][:, 128:384]
                S[i] = jnp.dot(lhs, rhs, preferred_element_type=f32)
            elif op == "S":
                sc = S.pop(i)
                m = jnp.max(sc, axis=1, keepdims=True)
                pf = jnp.exp2(sc - m).astype(bf).astype(f32)
                ps = pf[:, 0:128]
                for tt in range(1, SK // 128):
                    ps = ps + pf[:, tt * 128:(tt + 1) * 128]
                P[i] = (pf.astype(bf), 1.0 / jnp.sum(ps.T, axis=0, keepdims=True))
            elif op == "P":
                p, inv = P.pop(i)
                oT = lax.dot_general(vbuf[sl, i // 2, i % 2], p, NT, preferred_element_type=f32)
                O[i] = (oT * inv).astype(bf)
            else:
                o = jnp.concatenate([O.pop(2 * i), O.pop(2 * i + 1)], 0).T
                a = jnp.dot(o, wobuf[ws, i], preferred_element_type=f32)
                if not first:
                    a = jnp.where(hp == 0, 0.0, acc_ref[b, :, i * D:(i + 1) * D]) + a
                acc_ref[b, :, i * D:(i + 1) * D] = a
                obuf[b, :, i * D:(i + 1) * D] = a.astype(bf)
        if not first:
            pl.when(hp == NS - 1)(lambda: o_copy(b).start())

    x_copy(0, True).start(); wq_copy(0, 0).start(); kv_copy(0, 0, 0).start()
    x_copy(0, True).wait(); wq_copy(0, 0).wait()
    kv_copy(0, 0, 1).start()
    x_copy(1, True).start(); wq_copy(0, 1).start(); kv_copy(0, 1, 0).start()
    body(0, 0, True)

    def outer(hp, carry):
        @pl.when(hp > 0)
        def _():
            for s in range(2):
                wq_copy(hp, s).wait(); wo_copy(hp, s).wait()

        @pl.when(hp + 1 < NS)
        def _():
            for s in range(2):
                wq_copy(hp + 1, s).start(); wo_copy(hp + 1, s).start()

        def inner(b, carry):
            @pl.when(jnp.logical_and(hp == 0, b == 1))
            def _():
                for s in range(2): x_copy(s, False).wait()
            body(hp, b, False)
            return carry
        lax.fori_loop(jnp.where(hp == 0, 1, 0), B, inner, 0)
        return carry
    lax.fori_loop(0, NS, outer, 0)
    for b in range(B):
        o_copy(b).wait()


@jax.jit
def pallas_concat_heads__gqa_block_cached__gqa_block_cached__near_ridge_kernel(
        A_x, A_k_cache, A_v_cache, A_wq, A_wo, B_x, B_k_cache, B_v_cache, B_wq, B_wo):
    anyspec = pl.BlockSpec(memory_space=pl.ANY)
    tr = lambda a: jnp.swapaxes(a, 2, 3)
    return pl.pallas_call(
        _kernel,
        in_specs=[anyspec] * 10,
        out_specs=anyspec,
        out_shape=jax.ShapeDtypeStruct((B, SQ, 2 * D), bf),
        scratch_shapes=[pltpu.VMEM((2, B, SQ, D), bf),
                        pltpu.VMEM((2, 2, 2, DH, SK), bf), pltpu.VMEM((2, 2, 2, DH, SK), bf),
                        pltpu.VMEM((2, 2, D, W), bf), pltpu.VMEM((2, 2, W, D), bf),
                        pltpu.VMEM((B, SQ, 2 * D), f32), pltpu.VMEM((B, SQ, 2 * D), bf),
                        pltpu.SemaphoreType.DMA((2, 2)), pltpu.SemaphoreType.DMA((2, 2, 2)),
                        pltpu.SemaphoreType.DMA((2, 2, 2)), pltpu.SemaphoreType.DMA((B,))],
        compiler_params=pltpu.CompilerParams(vmem_limit_bytes=100 * 1024 * 1024),
    )(A_x, B_x, tr(A_k_cache), tr(A_v_cache), tr(B_k_cache), tr(B_v_cache), A_wq, B_wq, A_wo, B_wo)
```
